```python
import os as _os
_os.environ.setdefault("JAX_PLATFORMS", "cpu")
import jax
import jax.numpy as jnp

def _softmax(x, axis=-1):
    return jax.nn.softmax(x, axis=axis)
def _gelu(x):
    return jax.nn.gelu(x, approximate=True)
def _silu(x):
    return jax.nn.silu(x)
def _sigmoid(x):
    return jax.nn.sigmoid(x)
def _layernorm(x, axis=-1, eps=1e-5):
    m = jnp.mean(x, axis=axis, keepdims=True)
    v = jnp.var(x, axis=axis, keepdims=True)
    return (x - m) / jnp.sqrt(v + eps)
def _scatter_add(tgt, idx, src, axis=0):
    return tgt.at[idx].add(src)
def _segment_sum(src, seg, n):
    return jax.ops.segment_sum(src, seg, n)
class _Rng:
    def __init__(self, key):
        self._k = key
    def _next(self):
        self._k, sub = jax.random.split(self._k)
        return sub
    def normal(self, shape):
        return jax.random.normal(self._next(), shape, dtype=jnp.bfloat16)
    def randint(self, lo, hi, shape):
        return jax.random.randint(self._next(), shape, lo, hi, dtype=jnp.int32)
    def uniform(self, shape, lo=0.0, hi=1.0):
        return jax.random.uniform(self._next(), shape, jnp.bfloat16, lo, hi)
    def permutation(self, n):
        return jax.random.permutation(self._next(), n)


kernel_name = 'standalone__geglu_ffn__prompt'

def setup_inputs():
    _rng = _Rng(jax.random.key(int.from_bytes(__import__("os").urandom(4), "little")))
    _w = (lambda a: (lambda t: t.astype(jnp.bfloat16) if jnp.issubdtype(t.dtype, jnp.floating) else t)(jnp.asarray(a)))
    B, S, D, F = 1, 2048, 576, 4608
    return {
        "x": _w((lambda *s: _rng.normal(s) * 0.05)(B, S, D)),
        "w_gate": _w((lambda *s: _rng.normal(s) * 0.05)(D, F)),
        "w_up": _w((lambda *s: _rng.normal(s) * 0.05)(D, F)),
        "w_down": _w((lambda *s: _rng.normal(s) * 0.05)(F, D)),
    }

def reference(x, w_gate, w_up, w_down):
    return (_gelu(x @ w_gate) * (x @ w_up)) @ w_down
```

```python
import functools

import jax
import jax.experimental.pallas as pl
import jax.experimental.pallas.tpu as pltpu
import jax.numpy as jnp
import numpy as np
from jax import lax

_LANES = 128
_BM = 512
_HEAD = 256
_ROW_CUTS = (256, 384, 512, 768, 1024, 1536)
_COL_CUTS = (1024, 2304)
_LAST_SPLIT = 4

_C0 = float(np.sqrt(2.0 / np.pi))
_C1 = float(0.044715 * np.sqrt(2.0 / np.pi))

_GATE, _UP, _DOWN, _X = range(4)

_dot = functools.partial(jnp.dot, preferred_element_type=jnp.float32)


def _geglu(g, u):
    t = jnp.tanh(g * (_C0 + _C1 * (g * g)))
    return (0.5 * g * u) * (1.0 + t)


def _spans(edges):
    return list(zip(edges, edges[1:]))


def _block(m, start, n):
    if isinstance(m, int):
        return pl.ds(m * _BM + start, n)
    return pl.ds(pl.multiple_of(m * _BM + start, _LANES), n)


def _kernel(xt_hbm, wg_hbm, wu_hbm, wdt_hbm, ot_hbm, in_v, x_v, h0_v, o_v):
    d, s = xt_hbm.shape
    f = wg_hbm.shape[1]
    n_blocks = s // _BM
    n_tiles = _BM // _LANES
    slabs = _spans([*range(0, d, _LANES), d])
    row_spans = _spans([*_ROW_CUTS, s])
    col_spans = _spans([_HEAD, *_COL_CUTS, f])
    r0 = _ROW_CUTS[0]
    hbm = {_GATE: wg_hbm, _UP: wu_hbm, _DOWN: wdt_hbm, _X: xt_hbm}

    pieces = [(pl.ds(0, d), i) for i in range(n_tiles - 1)]
    step = d // _LAST_SPLIT
    pieces += [(pl.ds(j * step, step), n_tiles - 1) for j in range(_LAST_SPLIT)]

    def transpose_x(k0, k1, a, b):
        for i in range(a, b, _LANES):
            x_v[i : i + _LANES, k0:k1] = in_v[_X, k0:k1, i : i + _LANES].T

    def hidden(rows, a, b):
        xr = x_v[rows, :]
        g = _dot(xr, in_v[_GATE, :, a:b])
        u = _dot(xr, in_v[_UP, :, a:b])
        return _geglu(g, u).astype(h0_v.dtype)

    def run(in_sems, out_sem):
        n_groups = 0

        def fetch(*parts):
            nonlocal n_groups
            sem = in_sems.at[n_groups]
            n_groups += 1
            copies = [
                pltpu.make_async_copy(
                    hbm[w].at[k0:k1, a:b], in_v.at[w, k0:k1, a:b], sem
                )
                for w, k0, k1, a, b in parts
            ]
            for c in copies:
                c.start()

            def wait():
                for c in copies:
                    c.wait()

            return wait

        def store(m, rows, i):
            return pltpu.make_async_copy(
                o_v.at[m, rows, pl.ds(i * _LANES, _LANES)],
                ot_hbm.at[rows, _block(m, i * _LANES, _LANES)],
                out_sem,
            )

        wait_x0 = fetch((_X, *slabs[0], 0, r0))
        wait_slab = [
            fetch(
                *([(_X, k0, k1, 0, r0)] if k0 else []),
                (_GATE, k0, k1, 0, _HEAD),
                (_UP, k0, k1, 0, _HEAD),
            )
            for k0, k1 in slabs
        ]
        wait_rows = [fetch((_X, 0, d, a, b)) for a, b in row_spans]
        wait_cols = [fetch((_GATE, 0, d, a, b), (_UP, 0, d, a, b)) for a, b in col_spans]
        wait_down = fetch((_DOWN, 0, d, 0, f))

        wait_x0()
        transpose_x(*slabs[0], 0, r0)
        g = u = None
        for wait, (k0, k1) in zip(wait_slab, slabs):
            wait()
            if k0:
                transpose_x(k0, k1, 0, r0)
            xr = x_v[0:r0, k0:k1]
            pg = _dot(xr, in_v[_GATE, k0:k1, 0:_HEAD])
            g = pg if g is None else g + pg
            pu = _dot(xr, in_v[_UP, k0:k1, 0:_HEAD])
            u = pu if u is None else u + pu
        h0_v[0:r0, :] = _geglu(g, u).astype(h0_v.dtype)

        for wait, (a, b) in zip(wait_rows, row_spans):
            wait()
            for k0, k1 in slabs:
                transpose_x(k0, k1, a, b)
            h0_v[a:b, :] = hidden(slice(a, b), 0, _HEAD)

        def row_block(m, carry):
            on_first_trip = pl.when(m == 0)
            rows = _block(m, 0, _BM)
            hs = [h0_v[rows, :]]
            for wait, (a, b) in zip(wait_cols, col_spans):
                on_first_trip(wait)
                hs.append(hidden(rows, a, b))
            h = jnp.concatenate(hs, axis=1)
            on_first_trip(wait_down)
            for r, i in pieces:
                tile = slice(i * _LANES, (i + 1) * _LANES)
                out_t = lax.dot_general(
                    in_v[_DOWN, r, :],
                    h[tile, :],
                    (((1,), (1,)), ((), ())),
                    preferred_element_type=jnp.float32,
                )
                o_v[m, r, tile] = out_t.astype(o_v.dtype)
                store(m, r, i).start()
            return carry

        lax.fori_loop(0, n_blocks, row_block, None)
        for m in range(n_blocks):
            for r, i in pieces:
                store(m, r, i).wait()

    n_in = 1 + len(slabs) + len(row_spans) + len(col_spans) + 1
    pl.run_scoped(run, pltpu.SemaphoreType.DMA((n_in,)), pltpu.SemaphoreType.DMA(()))


@jax.jit
def pallas_standalone__geglu_ffn__prompt_kernel(
    x: jax.Array,
    w_gate: jax.Array,
    w_up: jax.Array,
    w_down: jax.Array,
):
    b, s, d = x.shape
    f = w_gate.shape[1]
    rows = b * s
    assert rows % _BM == 0 and _ROW_CUTS[-1] < rows <= f and f > _COL_CUTS[-1]

    in_hbm = pl.BlockSpec(memory_space=pl.ANY)
    out_t = pl.pallas_call(
        _kernel,
        in_specs=[in_hbm] * 4,
        out_specs=in_hbm,
        out_shape=jax.ShapeDtypeStruct((d, rows), x.dtype),
        scratch_shapes=[
            pltpu.VMEM((4, d, f), x.dtype),
            pltpu.VMEM((rows, d), x.dtype),
            pltpu.VMEM((rows, _HEAD), x.dtype),
            pltpu.VMEM((rows // _BM, d, _BM), x.dtype),
        ],
        compiler_params=pltpu.CompilerParams(
            vmem_limit_bytes=110 * 2**20,
            flags={"XLA_TPU_RESCHEDULE_DMA_DONES": True},
        ),
    )(x.reshape(rows, d).T, w_gate, w_up, w_down.T)
    return out_t.T.reshape(b, s, d)
```

```python
import functools

import jax
import jax.experimental.pallas as pl
import jax.experimental.pallas.tpu as pltpu
import jax.numpy as jnp
import numpy as np
from jax import lax

_LANES = 128
_BM = 512
_HEAD = 256
_ROW_CUTS = (256, 384, 512, 768, 1024, 1536)
_COL_CUTS = (1024, 2304)
_LAST_SPLIT = 4

_C0 = float(np.sqrt(2.0 / np.pi))
_C1 = float(0.044715 * np.sqrt(2.0 / np.pi))

_GATE, _UP, _DOWN, _X = range(4)

_dot = functools.partial(jnp.dot, preferred_element_type=jnp.float32)


def _geglu(g, u):
    t = jnp.tanh(g * (_C0 + _C1 * (g * g)))
    return (0.5 * g * u) * (1.0 + t)


def _spans(edges):
    return list(zip(edges, edges[1:]))


def _block(m, start, n):
    if isinstance(m, int):
        return pl.ds(m * _BM + start, n)
    return pl.ds(pl.multiple_of(m * _BM + start, _LANES), n)


def _kernel(xt_hbm, wg_hbm, wu_hbm, wdt_hbm, ot_hbm, in_v, x_v, h0_v, o_v):
    d, s = xt_hbm.shape
    f = wg_hbm.shape[1]
    n_blocks = s // _BM
    n_tiles = _BM // _LANES
    slabs = _spans([*range(0, d, _LANES), d])
    row_spans = _spans([*_ROW_CUTS, s])
    col_spans = _spans([_HEAD, *_COL_CUTS, f])
    r0 = _ROW_CUTS[0]
    hbm = {_GATE: wg_hbm, _UP: wu_hbm, _DOWN: wdt_hbm, _X: xt_hbm}

    pieces = [(pl.ds(0, d), i) for i in range(n_tiles - 1)]
    step = d // _LAST_SPLIT
    pieces += [(pl.ds(j * step, step), n_tiles - 1) for j in range(_LAST_SPLIT)]

    def transpose_x(k0, k1, a, b):
        for i in range(a, b, _LANES):
            x_v[i : i + _LANES, k0:k1] = in_v[_X, k0:k1, i : i + _LANES].T

    def hidden(rows, a, b):
        xr = x_v[rows, :]
        g = _dot(xr, in_v[_GATE, :, a:b])
        u = _dot(xr, in_v[_UP, :, a:b])
        return _geglu(g, u).astype(h0_v.dtype)

    def run(in_sems, out_sem):
        n_groups = 0

        def fetch(*parts):
            nonlocal n_groups
            sem = in_sems.at[n_groups]
            n_groups += 1
            copies = [
                pltpu.make_async_copy(
                    hbm[w].at[k0:k1, a:b], in_v.at[w, k0:k1, a:b], sem
                )
                for w, k0, k1, a, b in parts
            ]
            for c in copies:
                c.start()

            def wait():
                for c in copies:
                    c.wait()

            return wait

        def store(m, rows, i):
            return pltpu.make_async_copy(
                o_v.at[m, rows, pl.ds(i * _LANES, _LANES)],
                ot_hbm.at[rows, _block(m, i * _LANES, _LANES)],
                out_sem,
            )

        wait_x0 = fetch((_X, *slabs[0], 0, r0))
        wait_slab = [
            fetch(
                *([(_X, k0, k1, 0, r0)] if k0 else []),
                (_GATE, k0, k1, 0, _HEAD),
                (_UP, k0, k1, 0, _HEAD),
            )
            for k0, k1 in slabs
        ]
        wait_rows = [fetch((_X, 0, d, a, b)) for a, b in row_spans]
        wait_cols = [
            fetch((_GATE, 0, d, a, b), (_UP, 0, d, a, b)) for a, b in col_spans
        ]
        wait_down = fetch((_DOWN, 0, d, 0, f))

        def head():
            wait_x0()
            transpose_x(*slabs[0], 0, r0)
            g = u = None
            for wait, (k0, k1) in zip(wait_slab, slabs):
                wait()
                if k0:
                    transpose_x(k0, k1, 0, r0)
                xr = x_v[0:r0, k0:k1]
                pg = _dot(xr, in_v[_GATE, k0:k1, 0:_HEAD])
                g = pg if g is None else g + pg
                pu = _dot(xr, in_v[_UP, k0:k1, 0:_HEAD])
                u = pu if u is None else u + pu
            h0_v[0:r0, :] = _geglu(g, u).astype(h0_v.dtype)

            for wait, (a, b) in zip(wait_rows, row_spans):
                wait()
                for k0, k1 in slabs:
                    transpose_x(k0, k1, a, b)
                h0_v[a:b, :] = hidden(slice(a, b), 0, _HEAD)

        def row_block(m, carry):
            on_first_trip = pl.when(m == 0)
            on_first_trip(head)
            rows = _block(m, 0, _BM)
            hs = [h0_v[rows, :]]
            for wait, (a, b) in zip(wait_cols, col_spans):
                on_first_trip(wait)
                hs.append(hidden(rows, a, b))
            h = jnp.concatenate(hs, axis=1)
            on_first_trip(wait_down)
            for r, i in pieces:
                tile = slice(i * _LANES, (i + 1) * _LANES)
                out_t = lax.dot_general(
                    in_v[_DOWN, r, :],
                    h[tile, :],
                    (((1,), (1,)), ((), ())),
                    preferred_element_type=jnp.float32,
                )
                o_v[m, r, tile] = out_t.astype(o_v.dtype)
                store(m, r, i).start()
            return carry

        lax.fori_loop(0, n_blocks, row_block, None)
        for m in range(n_blocks):
            for r, i in pieces:
                store(m, r, i).wait()

    n_in = 1 + len(slabs) + len(row_spans) + len(col_spans) + 1
    pl.run_scoped(run, pltpu.SemaphoreType.DMA((n_in,)), pltpu.SemaphoreType.DMA(()))


@jax.jit
def pallas_standalone__geglu_ffn__prompt_kernel(
    x: jax.Array,
    w_gate: jax.Array,
    w_up: jax.Array,
    w_down: jax.Array,
):
    b, s, d = x.shape
    f = w_gate.shape[1]
    rows = b * s
    assert rows % _BM == 0 and _ROW_CUTS[-1] < rows <= f and f > _COL_CUTS[-1]

    in_hbm = pl.BlockSpec(memory_space=pl.ANY)
    out_t = pl.pallas_call(
        _kernel,
        in_specs=[in_hbm] * 4,
        out_specs=in_hbm,
        out_shape=jax.ShapeDtypeStruct((d, rows), x.dtype),
        scratch_shapes=[
            pltpu.VMEM((4, d, f), x.dtype),
            pltpu.VMEM((rows, d), x.dtype),
            pltpu.VMEM((rows, _HEAD), x.dtype),
            pltpu.VMEM((rows // _BM, d, _BM), x.dtype),
        ],
        compiler_params=pltpu.CompilerParams(
            vmem_limit_bytes=110 * 2**20,
            flags={"XLA_TPU_RESCHEDULE_DMA_DONES": True},
        ),
    )(x.reshape(rows, d).T, w_gate, w_up, w_down.T)
    return out_t.T.reshape(b, s, d)
```
